```python
import os as _os
_os.environ.setdefault("JAX_PLATFORMS", "cpu")
import jax
import jax.numpy as jnp

def _softmax(x, axis=-1):
    return jax.nn.softmax(x, axis=axis)
def _gelu(x):
    return jax.nn.gelu(x, approximate=True)
def _silu(x):
    return jax.nn.silu(x)
def _sigmoid(x):
    return jax.nn.sigmoid(x)
def _layernorm(x, axis=-1, eps=1e-5):
    m = jnp.mean(x, axis=axis, keepdims=True)
    v = jnp.var(x, axis=axis, keepdims=True)
    return (x - m) / jnp.sqrt(v + eps)
def _scatter_add(tgt, idx, src, axis=0):
    return tgt.at[idx].add(src)
def _segment_sum(src, seg, n):
    return jax.ops.segment_sum(src, seg, n)
class _Rng:
    def __init__(self, key):
        self._k = key
    def _next(self):
        self._k, sub = jax.random.split(self._k)
        return sub
    def normal(self, shape):
        return jax.random.normal(self._next(), shape, dtype=jnp.bfloat16)
    def randint(self, lo, hi, shape):
        return jax.random.randint(self._next(), shape, lo, hi, dtype=jnp.int32)
    def uniform(self, shape, lo=0.0, hi=1.0):
        return jax.random.uniform(self._next(), shape, jnp.bfloat16, lo, hi)
    def permutation(self, n):
        return jax.random.permutation(self._next(), n)


kernel_name = 'standalone__linear_kernel_rfa__decode'

def setup_inputs():
    _rng = _Rng(jax.random.key(int.from_bytes(__import__("os").urandom(4), "little")))
    _w = (lambda a: (lambda t: t.astype(jnp.bfloat16) if jnp.issubdtype(t.dtype, jnp.floating) else t)(jnp.asarray(a)))
    B, H, Sq, Sk, D, M = 2, 16, 1, 16384, 256, 16
    return {
        "q": _w((lambda *s: _rng.normal(s) * 0.4)(B, H, Sq, D)),
        "k": _w((lambda *s: _rng.normal(s) * 1.6)(B, H, Sk, D)),
        "v": _w((lambda *s: _rng.normal(s) * 1.6)(B, H, Sk, D)),
        "omega": _w((lambda *s: _rng.normal(s) * 1.6)(M, D)),
    }

def reference(q, k, v, omega):
    d = q.shape[-1]
    m = omega.shape[0]
    scale = float(d) ** -0.25
    qs = q * scale
    ks = k * scale
    q_proj = jnp.einsum("bhsd,md->bhsm", qs, omega)
    k_proj = jnp.einsum("bhsd,md->bhsm", ks, omega)
    q_sq = 0.5 * jnp.einsum("bhsd,bhsd->bhs", qs, qs)[..., None]
    k_sq = 0.5 * jnp.einsum("bhsd,bhsd->bhs", ks, ks)[..., None]
    inv_sqrt_m = float(m) ** -0.5
    phi_q = jnp.exp(q_proj - q_sq) * inv_sqrt_m + 1e-6
    phi_k = jnp.exp(k_proj - k_sq) * inv_sqrt_m + 1e-6
    kv = jnp.einsum("bhsm,bhsd->bhmd", phi_k, v)
    z  = jnp.einsum("bhsm->bhm", phi_k)
    num = jnp.einsum("bhqm,bhmd->bhqd", phi_q, kv)
    den = jnp.einsum("bhqm,bhm->bhq", phi_q, z)[..., None] + 1e-6
    return num / den
```

```python
import functools

import jax
import jax.numpy as jnp
import jax.experimental.pallas as pl
import jax.experimental.pallas.tpu as pltpu

_NT = (((1,), (1,)), ((), ()))
_BLOCK_S = 1024
_LANES = 128


def _rfa_kernel(q_ref, om_ref, k_ref, v_ref, o_ref, kv_acc, z_acc, o_acc, *,
                scale, inv_sqrt_m):
    head = pl.program_id(0)
    j = pl.program_id(1)
    half = k_ref.shape[-1] // 2

    @pl.when(j == 0)
    def _():
        kv_acc[...] = jnp.zeros_like(kv_acc)
        z_acc[...] = jnp.zeros_like(z_acc)

    om = om_ref[...]
    k = k_ref[...]
    proj = jax.lax.dot_general(om, k, _NT, preferred_element_type=jnp.float32)
    kf = k.astype(jnp.float32)
    sq = kf[:, :half] * kf[:, :half] + kf[:, half:] * kf[:, half:]
    ones = jnp.ones((om.shape[0], half), jnp.bfloat16)
    ksq = jax.lax.dot_general(ones, sq.astype(jnp.bfloat16), _NT,
                              preferred_element_type=jnp.float32)
    phi = jnp.exp(proj * scale - ksq * (0.5 * scale * scale)) * inv_sqrt_m + 1e-6
    pb = phi.astype(jnp.bfloat16)
    kv_acc[...] += jnp.dot(pb, v_ref[...], preferred_element_type=jnp.float32)
    pf = pb.astype(jnp.float32)
    zs = pf[:, :_LANES]
    for t in range(1, pf.shape[1] // _LANES):
        zs = zs + pf[:, t * _LANES:(t + 1) * _LANES]
    z_acc[...] += zs

    @pl.when(j == pl.num_programs(1) - 1)
    def _():
        qf = q_ref[...].astype(jnp.float32)
        rows = jax.lax.broadcasted_iota(jnp.int32, qf.shape, 0)
        qf = jnp.sum(jnp.where(rows == head, qf, 0.0), axis=0, keepdims=True)
        omf = om.astype(jnp.float32)
        q_proj = jnp.sum(omf * qf, axis=-1, keepdims=True) * scale
        q_sq = jnp.sum(qf * qf, axis=-1, keepdims=True) * (0.5 * scale * scale)
        phi_q = jnp.exp(q_proj - q_sq) * inv_sqrt_m + 1e-6
        num = jnp.sum(phi_q * kv_acc[...], axis=0, keepdims=True)
        z = jnp.sum(z_acc[...], axis=-1, keepdims=True)
        den = jnp.sum(phi_q * z, axis=0, keepdims=True) + 1e-6
        o_acc[pl.ds(head, 1), :] = num / den

        @pl.when(head == pl.num_programs(0) - 1)
        def _():
            o_ref[...] = o_acc[...].astype(o_ref.dtype)


@jax.jit
def pallas_standalone__linear_kernel_rfa__decode_kernel(q, k, v, omega):
    b, h, sq, d = q.shape
    sk = k.shape[2]
    m = omega.shape[0]
    bs = _BLOCK_S
    assert sq == 1 and sk % bs == 0 and d % (2 * _LANES) == 0
    nh = b * h
    body = functools.partial(
        _rfa_kernel, scale=float(d) ** -0.25, inv_sqrt_m=float(m) ** -0.5)
    out = pl.pallas_call(
        body,
        grid=(nh, sk // bs),
        in_specs=[
            pl.BlockSpec((nh, d), lambda i, j: (0, 0)),
            pl.BlockSpec((m, d), lambda i, j: (0, 0)),
            pl.BlockSpec((None, bs, d), lambda i, j: (i, j, 0)),
            pl.BlockSpec((None, bs, d), lambda i, j: (i, j, 0)),
        ],
        out_specs=pl.BlockSpec((nh, d), lambda i, j: (0, 0)),
        out_shape=jax.ShapeDtypeStruct((nh, d), q.dtype),
        scratch_shapes=[
            pltpu.VMEM((m, d), jnp.float32),
            pltpu.VMEM((m, _LANES), jnp.float32),
            pltpu.VMEM((nh, d), jnp.float32),
        ],
        compiler_params=pltpu.CompilerParams(
            dimension_semantics=("arbitrary", "arbitrary"),
            vmem_limit_bytes=64 * 1024 * 1024,
        ),
    )(q.reshape(nh, d), omega, k.reshape(nh, sk, d), v.reshape(nh, sk, d))
    return out.reshape(b, h, sq, d)
```

```python
import functools

import jax
import jax.numpy as jnp
import jax.experimental.pallas as pl
import jax.experimental.pallas.tpu as pltpu

_NT = (((1,), (1,)), ((), ()))
_LANES = 128
_CHUNK = 1024
_DMA_ROWS = 64
_NBUF = 6
_V_ROT = 2


def _rfa_kernel(q_ref, om_ref, k_hbm, v_hbm, o_ref, kb, vb, o_acc, sem, *,
                scale, inv_sqrt_m):
    nh, seq, d = k_hbm.shape
    m = om_ref.shape[0]
    half = d // 2
    nc = seq // _CHUNK
    total = nh * nc
    pieces = _CHUNK // _DMA_ROWS

    def start(i):
        h, c, slot = i // nc, i % nc, i % _NBUF
        for s in range(pieces):
            r = (s + _V_ROT) % pieces
            pltpu.make_async_copy(
                k_hbm.at[h, pl.ds(c * _CHUNK + s * _DMA_ROWS, _DMA_ROWS)],
                kb.at[slot, pl.ds(s * _DMA_ROWS, _DMA_ROWS)],
                sem.at[0, slot]).start(priority=0)
            pltpu.make_async_copy(
                v_hbm.at[h, pl.ds(c * _CHUNK + r * _DMA_ROWS, _DMA_ROWS)],
                vb.at[slot, pl.ds(r * _DMA_ROWS, _DMA_ROWS)],
                sem.at[1, slot]).start(priority=1)

    def wait(buf, which, slot):
        pltpu.make_async_copy(buf.at[slot], buf.at[slot],
                              sem.at[which, slot]).wait()

    for i in range(_NBUF - 1):
        start(i)

    om = om_ref[...]
    omf = om.astype(jnp.float32)
    qf = q_ref[...].astype(jnp.float32)
    ones = jnp.ones((m, half), jnp.bfloat16)
    half_s2 = 0.5 * scale * scale

    def head(h, _):
        rows = jax.lax.broadcasted_iota(jnp.int32, qf.shape, 0)
        qh = jnp.sum(jnp.where(rows == h, qf, 0.0), axis=0, keepdims=True)
        q_proj = jnp.sum(omf * qh, axis=-1, keepdims=True) * scale
        q_sq = jnp.sum(qh * qh, axis=-1, keepdims=True) * half_s2
        phi_q = jnp.exp(q_proj - q_sq) * inv_sqrt_m + 1e-6

        def chunk(c, carry):
            kv, z = carry
            i = h * nc + c
            slot = i % _NBUF
            nxt = i + _NBUF - 1
            pl.when(nxt < total)(lambda: start(nxt))

            wait(kb, 0, slot)
            k = kb[slot]
            proj = jax.lax.dot_general(om, k, _NT,
                                       preferred_element_type=jnp.float32)
            kf = k.astype(jnp.float32)
            sq = kf[:, :half] * kf[:, :half] + kf[:, half:] * kf[:, half:]
            ksq = jax.lax.dot_general(ones, sq.astype(jnp.bfloat16), _NT,
                                      preferred_element_type=jnp.float32)
            phi = jnp.exp(proj * scale - ksq * half_s2) * inv_sqrt_m + 1e-6
            pb = phi.astype(jnp.bfloat16)
            pf = pb.astype(jnp.float32)
            zs = pf[:, :_LANES]
            for t in range(1, _CHUNK // _LANES):
                zs = zs + pf[:, t * _LANES:(t + 1) * _LANES]

            wait(vb, 1, slot)
            kv = kv + jnp.dot(pb, vb[slot], preferred_element_type=jnp.float32)
            return kv, z + zs

        kv, z = jax.lax.fori_loop(
            0, nc, chunk,
            (jnp.zeros((m, d), jnp.float32), jnp.zeros((m, _LANES), jnp.float32)))
        num = jnp.sum(phi_q * kv, axis=0, keepdims=True)
        zz = jnp.sum(z, axis=-1, keepdims=True)
        den = jnp.sum(phi_q * zz, axis=0, keepdims=True) + 1e-6
        o_acc[pl.ds(h, 1), :] = num / den

    jax.lax.fori_loop(0, nh, head, None)
    o_ref[...] = o_acc[...].astype(o_ref.dtype)


@jax.jit
def pallas_standalone__linear_kernel_rfa__decode_kernel(q, k, v, omega):
    b, h, sq, d = q.shape
    sk = k.shape[2]
    m = omega.shape[0]
    nh = b * h
    assert sq == 1 and sk % _CHUNK == 0 and d % (2 * _LANES) == 0
    assert nh * (sk // _CHUNK) >= _NBUF
    body = functools.partial(
        _rfa_kernel, scale=float(d) ** -0.25, inv_sqrt_m=float(m) ** -0.5)
    out = pl.pallas_call(
        body,
        in_specs=[
            pl.BlockSpec(memory_space=pltpu.VMEM),
            pl.BlockSpec(memory_space=pltpu.VMEM),
            pl.BlockSpec(memory_space=pl.ANY),
            pl.BlockSpec(memory_space=pl.ANY),
        ],
        out_specs=pl.BlockSpec(memory_space=pltpu.VMEM),
        out_shape=jax.ShapeDtypeStruct((nh, d), q.dtype),
        scratch_shapes=[
            pltpu.VMEM((_NBUF, _CHUNK, d), k.dtype),
            pltpu.VMEM((_NBUF, _CHUNK, d), v.dtype),
            pltpu.VMEM((nh, d), jnp.float32),
            pltpu.SemaphoreType.DMA((2, _NBUF)),
        ],
        compiler_params=pltpu.CompilerParams(
            vmem_limit_bytes=64 * 1024 * 1024),
    )(q.reshape(nh, d), omega, k.reshape(nh, sk, d), v.reshape(nh, sk, d))
    return out.reshape(b, h, sq, d)
```
